```python
import jax
import jax.numpy as jnp

def _softmax(x, axis=-1):
    return jax.nn.softmax(x, axis=axis)

def _gelu(x):
    return jax.nn.gelu(x, approximate=True)

def _silu(x):
    return jax.nn.silu(x)

def _sigmoid(x):
    return jax.nn.sigmoid(x)

def _layernorm(x, axis=-1, eps=1e-05):
    m = jnp.mean(x, axis=axis, keepdims=True)
    v = jnp.var(x, axis=axis, keepdims=True)
    return (x - m) / jnp.sqrt(v + eps)

def _scatter_add(tgt, idx, src, axis=0):
    return tgt.at[idx].add(src)

def _segment_sum(src, seg, n):
    return jax.ops.segment_sum(src, seg, n)

class _Rng:

    def __init__(self, key):
        self._k = key

    def _next(self):
        self._k, sub = jax.random.split(self._k)
        return sub

    def normal(self, shape):
        return jax.random.normal(self._next(), shape, dtype=jnp.bfloat16)

    def randint(self, lo, hi, shape):
        return jax.random.randint(self._next(), shape, lo, hi, dtype=jnp.int32)

    def uniform(self, shape, lo=0.0, hi=1.0):
        return jax.random.uniform(self._next(), shape, jnp.bfloat16, lo, hi)

    def permutation(self, n):
        return jax.random.permutation(self._next(), n)
kernel_name = 'parallel_sum__mha_block__mixer_gmlp__prompt'

def _fwd_setup_inputs():
    _rng = _Rng(jax.random.key(int.from_bytes(__import__("os").urandom(4), "little")))
    _w = lambda a: (lambda t: t.astype(jnp.bfloat16) if jnp.issubdtype(t.dtype, jnp.floating) else t)(jnp.asarray(a))

    def _A_setup():
        B, S, D, H = (1, 2048, 1024, 32)
        return {'x': _w((lambda *s: _rng.normal(s) * 0.05)(B, S, D)), 'wqkv': _w((lambda *s: _rng.normal(s) * 0.05)(D, 3 * D)), 'wo': _w((lambda *s: _rng.normal(s) * 0.05)(D, D))}
    _A_in = _A_setup()

    def _B_setup():
        B, S, D, F = (1, 2048, 1024, 3584)
        Fh = F // 2
        return {'x': _w((lambda *s: _rng.normal(s) * 0.05)(B, S, D)), 'w_in': _w((lambda *s: _rng.normal(s) * 0.05)(D, 2 * Fh)), 'w_sp': _w(0.01 * (lambda *s: _rng.normal(s) * 0.05)(S, S)), 'b_sp': _w(1.0 + 0.01 * (lambda *s: _rng.normal(s) * 0.05)(S)), 'w_out': _w((lambda *s: _rng.normal(s) * 0.05)(Fh, D))}
    _B_in = _B_setup()
    return {'A_x': _A_in['x'], 'A_wqkv': _A_in['wqkv'], 'A_wo': _A_in['wo'], 'B_x': _B_in['x'], 'B_w_in': _B_in['w_in'], 'B_w_sp': _B_in['w_sp'], 'B_b_sp': _B_in['b_sp'], 'B_w_out': _B_in['w_out']}

def _fwd_reference(A_x, A_wqkv, A_wo, B_x, B_w_in, B_w_sp, B_b_sp, B_w_out):

    def _A_ref(x, wqkv, wo):
        B, S, D = x.shape
        H = 32
        Dh = D // H
        qkv = (lambda x, *d: x.transpose(*d))((x @ wqkv).reshape(B, S, 3, H, Dh), 2, 0, 3, 1, 4)
        q, k, v = (qkv[0], qkv[1], qkv[2])
        scores = jnp.einsum('bhqd,bhkd->bhqk', q, k) * Dh ** (-0.5)
        p = _softmax(scores, axis=-1)
        o = jnp.einsum('bhqk,bhkd->bhqd', p, v)
        return (lambda x, *d: x.transpose(*d))(o, 0, 2, 1, 3).reshape(B, S, D) @ wo

    def _B_ref(x, w_in, w_sp, b_sp, w_out):
        B, S, D = x.shape
        F = w_in.shape[-1]
        Fh = F // 2
        z = _gelu(jnp.einsum('bsd,df->bsf', x, w_in))
        z1 = z[..., :Fh].copy()
        z2 = _layernorm(z[..., Fh:], axis=-1)
        g = jnp.einsum('ts,bsf->btf', w_sp, z2) + b_sp[None, :, None]
        return jnp.einsum('bsf,fd->bsd', z1 * g, w_out)
    x = A_x
    xn = _layernorm(x, axis=-1)
    return x + _A_ref(xn, A_wqkv, A_wo) + _B_ref(xn, B_w_in, B_w_sp, B_b_sp, B_w_out)

def setup_inputs():
    _inp = _fwd_setup_inputs()
    _gk = jax.random.fold_in(jax.random.key(int.from_bytes(__import__("os").urandom(4), "little")), 2 ** 31 - 1)
    _shapes = [[1, 2048, 1024]]
    _dtypes = ['bfloat16']
    _gks = jax.random.split(_gk, len(_shapes))
    _gs = [jax.random.normal(k, s, dtype=jnp.dtype(d)) * 0.05 for k, s, d in zip(_gks, _shapes, _dtypes)]
    _inp['grad_out'] = _gs[0]
    return _inp

def reference(A_x, A_wqkv, A_wo, B_w_in, B_w_sp, B_b_sp, B_w_out, B_x, grad_out):
    _const = dict(B_x=B_x)

    def _f(*_d):
        return _fwd_reference(**{'A_x': _d[0], 'A_wqkv': _d[1], 'A_wo': _d[2], 'B_w_in': _d[3], 'B_w_sp': _d[4], 'B_b_sp': _d[5], 'B_w_out': _d[6], **_const})
    _out, _vjp = jax.vjp(_f, A_x, A_wqkv, A_wo, B_w_in, B_w_sp, B_b_sp, B_w_out)
    _grads = _vjp(grad_out)
    _out0 = jnp.asarray(_out)
    return (_out0, *[jnp.asarray(_g) for _g in _grads])
```

```python
import functools
import math

import jax
import jax.numpy as jnp
from jax import lax
import jax.experimental.pallas as pl
import jax.experimental.pallas.tpu as pltpu

S = 2048
D = 1024
H = 32
DH = 32
F = 3584
FH = F // 2
EPS = 1e-5

bf = jnp.bfloat16
f32 = jnp.float32
u32 = jnp.uint32

NN = (((1,), (0,)), ((), ()))
NT = (((1,), (1,)), ((), ()))

LN2 = math.log(2.0)
SCALE = DH ** -0.5
GELU_C = math.sqrt(2.0 / math.pi)
GELU_A = 0.044715

MQ = 512
KC = 128
NCH = S // KC
NQB = S // MQ
NBLK = H * NQB
DB = 2
DA = 4
ATT_ITERS = (NBLK + 4) // 2


def _dot(a, b, dims):
    return lax.dot_general(a, b, dims, preferred_element_type=f32)


def _tobf(x):
    return pltpu.bitcast(x, bf)


def _tou(x):
    return pltpu.bitcast(x, u32)


def _r3(x):
    return x.reshape(x.shape[0] // 8, 8, x.shape[1])


def _sub8(x, row8):
    return (_r3(x) - row8[None]).reshape(x.shape)


def _ds(i, n):
    return pl.ds(pl.multiple_of(i * n, n), n)


def _rowmean(x):
    return jnp.sum(x, axis=-1, keepdims=True) * (1.0 / x.shape[-1])


def _ln_stats(xf):
    m = _rowmean(xf)
    xc = xf - m
    v = _rowmean(xc * xc)
    rstd = lax.rsqrt(v + EPS)
    return xc * rstd, rstd


def _gelu_and_grad(x):
    x2 = x * x
    t = jnp.tanh(GELU_C * (x + GELU_A * (x2 * x)))
    h = 0.5 * (1.0 + t)
    g = x * h
    dg = h + (0.5 * GELU_C) * x * (1.0 - t * t) * (1.0 + (3.0 * GELU_A) * x2)
    return g, dg


SEM_WO = 0
SEM_X = 1
SEM_DOUT = 9
SEM_WQKV = 17
SEM_WIN = 18
SEM_WSP = 19
SEM_WOUT = 20
SEM_ST = 21
NSEM = 25


def _kernel(x_hbm, wqkv_hbm, wo_hbm, win_hbm, wsp_hbm, bsp_ref, wout_hbm, dout_hbm,
            out_hbm, dx_hbm, dwqkv_hbm, dwo_hbm, dwin_hbm, dwsp_hbm, dbsp_ref, dwout_hbm,
            x_v, dout_v, wo_v, win_v, xn_v, xnT_v, onat_v, dxa_v, sems):

    def in_copy(src, dst, s):
        return pltpu.make_async_copy(src, dst, sems.at[s])

    def x_copy(i):
        return in_copy(x_hbm.at[_ds(i, 256)], x_v.at[_ds(i, 256)], SEM_X + i)

    def dout_copy(i):
        return in_copy(dout_hbm.at[_ds(i, 256)], dout_v.at[_ds(i, 256)], SEM_DOUT + i)

    def stream_out(n_iters, stage, dst_fn, sem0):
        def cp(i, slot):
            return pltpu.make_async_copy(stage.at[slot], dst_fn(i), sems.at[sem0 + slot])

        def acquire(i):
            @pl.when(i >= 2)
            def _():
                cp(i - 2, i % 2).wait()

        def release(i):
            cp(i, i % 2).start()

        def drain():
            cp(n_iters - 2, n_iters % 2).wait()
            cp(n_iters - 1, (n_iters - 1) % 2).wait()

        return acquire, release, drain

    def scope_a(wqkv_v, kv_v, qkvT_v, dOT_v, oT_v, dqkvT_v):
        in_copy(wo_hbm, wo_v, SEM_WO).start()
        for i in range(8):
            dout_copy(i).start()
            x_copy(i).start()
        in_copy(wqkv_hbm, wqkv_v, SEM_WQKV).start()
        in_copy(win_hbm, win_v, SEM_WIN).start()

        in_copy(wo_hbm, wo_v, SEM_WO).wait()

        def phase_d(i, c):
            dout_copy(i).wait()
            x_copy(i).wait()
            rows = _ds(i, 256)
            dOT_v[:, rows] = _tou(_dot(wo_v[...], dout_v[rows, :], NT).astype(bf))
            xn, _ = _ln_stats(x_v[rows, :].astype(f32))
            xnb = xn.astype(bf)
            xn_v[_ds(i, 128), :] = _tou(xnb)
            xnT_v[:, rows] = _tou(xnb.T)
            return c

        lax.fori_loop(0, 8, phase_d, 0)

        in_copy(wqkv_hbm, wqkv_v, SEM_WQKV).wait()

        def phase_q(i, c):
            rows = _ds(i, 256)
            xnb = _tobf(xn_v[_ds(i, 128), :])
            for n in (2, 3, 4, 5, 0, 1):
                r = _dot(xnb, wqkv_v[:, n * 512:(n + 1) * 512], NN)
                if n < 2:
                    r = r * (SCALE / LN2)
                rb = r.astype(bf)
                if n >= 2:
                    ru = _tou(rb)
                    for p in range(4):
                        kv_v[(n - 2) * 4 + p, _ds(i, 128), :] = ru[:, p * 128:(p + 1) * 128]
                qkvT_v[n * 256:(n + 1) * 256, rows] = _tou(rb.T)
            return c

        lax.fori_loop(0, 8, phase_q, 0)

        def attention(s_buf0, s_buf1, p_buf0, p_buf1, m_buf, dos_buf, dl_buf, dk_acc, dv_acc):
            for r in (s_buf0, s_buf1, p_buf0, p_buf1, m_buf, dos_buf, dl_buf, dk_acc, dv_acc):
                r[...] = jnp.zeros_like(r)
            s_bufs = (s_buf0, s_buf1)
            p_bufs = (p_buf0, p_buf1)
            lane_h = lax.broadcasted_iota(jnp.int32, (64, 128), 1) // 32

            def bc8(v):
                return jnp.broadcast_to(v, (8, MQ))

            def dec(b, par):
                b = jnp.clip(b, 0, NBLK - 1)
                h = b // NQB
                qb = b % NQB
                return dict(h=h, qb=qb, g=h // 4, r=h % 4, qo=pl.multiple_of(qb * MQ, MQ), s=par)

            def row16(base, h):
                return pl.ds(pl.multiple_of(base + h * 16, 16), 16)

            def body(it, carry):
                m_run, l_run, ot_acc = carry
                t0 = it * 2 - 4
                blks = [dec(t0 + i, i % 2) for i in range(5)]
                pend_dk = None
                pend_o = None

                def do_dkdq(c, j, dsb):
                    ks = slice(j * KC, (j + 1) * KC)
                    dkp = _dot(c['qT'], dsb, NT)
                    dk_new = dk_acc[:, ks]
                    if c['s'] == 0:
                        dk_new = jnp.where(c['qb'] == 0, 0.0, dk_new)
                    dk_new = dk_new + dkp
                    dk_acc[:, ks] = dk_new
                    if c['s'] == 1:
                        dqkvT_v[row16(512, c['h']), ks] = _tou((dk_new * LN2).astype(bf))
                    kT = _tobf(qkvT_v[row16(512, c['h']), ks])
                    dq = _dot(kT, dsb, NN)
                    c['dq'] = dq if j == 0 else c['dq'] + dq
                    if j == NCH - 1:
                        dqkvT_v[row16(0, c['h']), pl.ds(c['qo'], MQ)] = _tou((c['dq'] * SCALE).astype(bf))

                def do_o(b, j, pbn, ot_acc):
                    ks = slice(j * KC, (j + 1) * KC)
                    vT = _tobf(qkvT_v[row16(1024, b['h']), ks])
                    o = _dot(vT, pbn, NN)
                    return o if j == 0 else ot_acc + o

                for u in range(2):
                    c = blks[u]
                    b0 = blks[u + 1]
                    b1 = blks[u + 2]
                    a0 = blks[u + 2]
                    a1 = blks[u + 3]
                    dosT = _tobf(dos_buf[c['s']])
                    dos4 = jnp.concatenate([dosT] * 4, axis=0)
                    dl = dl_buf[c['s']]
                    c['qT'] = _tobf(qkvT_v[row16(0, c['h']), pl.ds(c['qo'], MQ)])
                    for j in range(NCH):
                        ks = slice(j * KC, (j + 1) * KC)
                        ksu = slice(j * 64, (j + 1) * 64)
                        v4 = _tobf(jnp.where(lane_h == c['r'], kv_v[8 + c['g'], ksu, :], jnp.uint32(0)))
                        dpT = _dot(v4, dos4, NN)
                        pb = _tobf(p_bufs[c['s']][ksu, :])
                        dvp = _dot(dosT, pb, NT)
                        dv_new = dv_acc[:, ks]
                        if c['s'] == 0:
                            dv_new = jnp.where(c['qb'] == 0, 0.0, dv_new)
                        dv_new = dv_new + dvp
                        dv_acc[:, ks] = dv_new
                        if c['s'] == 1:
                            dqkvT_v[row16(1024, c['h']), ks] = _tou(dv_new.astype(bf))
                        dsb = (pb.astype(f32) * _sub8(dpT, dl)).astype(bf)
                        if pend_dk is not None:
                            do_dkdq(*pend_dk)
                        pend_dk = (c, j, dsb)
                        ja = (j + DA) % NCH
                        a = a0 if j + DA < NCH else a1
                        kau = slice(ja * 64, (ja + 1) * 64)
                        k4 = _tobf(jnp.where(lane_h == a['r'], kv_v[a['g'], kau, :], jnp.uint32(0)))
                        qT4 = _tobf(qkvT_v[pl.ds(pl.multiple_of(a['g'] * 64, 64), 64), pl.ds(a['qo'], MQ)])
                        sT = _dot(k4, qT4, NN)
                        s_bufs[a['s']][ja * KC:(ja + 1) * KC, :] = sT
                        cm = jnp.max(_r3(sT), axis=0)
                        m_run = cm if ja == 0 else jnp.maximum(m_run, cm)
                        if ja == NCH - 1:
                            m_buf[a['s']] = bc8(jnp.max(m_run, axis=0, keepdims=True))
                        if pend_o is not None:
                            ot_acc = do_o(*pend_o, ot_acc)
                            if pend_o[1] == NCH - 1:
                                l = jnp.sum(l_run, axis=0, keepdims=True)
                                rl = 1.0 / l
                                ot = ot_acc * rl
                                oT_v[row16(0, b0['h']), pl.ds(b0['qo'], MQ)] = _tou(ot.astype(bf))
                                dob = _tobf(dOT_v[row16(0, b0['h']), pl.ds(b0['qo'], MQ)]).astype(f32) * rl
                                dos_buf[b0['s']] = _tou(dob.astype(bf))
                                dl_buf[b0['s']] = bc8(jnp.sum(dob * ot, axis=0, keepdims=True))
                        jb = (j + DB) % NCH
                        b = b0 if j + DB < NCH else b1
                        mb = m_buf[b['s']]
                        mb = jnp.where(mb != mb, cm, mb)
                        p = jnp.exp2(_sub8(s_bufs[b['s']][jb * KC:(jb + 1) * KC, :], mb))
                        ps = jnp.sum(_r3(p), axis=0)
                        l_run = ps if jb == 0 else l_run + ps
                        pbn = p.astype(bf)
                        p_bufs[b['s']][jb * 64:(jb + 1) * 64, :] = _tou(pbn)
                        pend_o = (b, jb, pbn)
                do_dkdq(*pend_dk)
                ot_acc = do_o(*pend_o, ot_acc)
                return m_run, l_run, ot_acc

            init = (jnp.zeros((8, MQ), f32), jnp.ones((8, MQ), f32), jnp.zeros((32, MQ), f32))
            lax.fori_loop(0, ATT_ITERS, body, init)

        pl.run_scoped(
            attention,
            pltpu.VMEM((S, MQ), f32), pltpu.VMEM((S, MQ), f32),
            pltpu.VMEM((S // 2, MQ), u32), pltpu.VMEM((S // 2, MQ), u32),
            pltpu.VMEM((2, 8, MQ), f32), pltpu.VMEM((2, 16, MQ), u32), pltpu.VMEM((2, 8, MQ), f32),
            pltpu.VMEM((32, S), f32), pltpu.VMEM((32, S), f32),
        )

        def post_a(st_wo, st_wqkv):
            acq, rel, drain = stream_out(4, st_wo, lambda i: dwo_hbm.at[_ds(i, 256)], SEM_ST)

            def phase_wo(i, c):
                acq(i)
                oTb = _tobf(oT_v[_ds(i, 128), :])
                st_wo[i % 2] = _dot(oTb, dout_v[...], NN).astype(bf)
                onat_v[:, _ds(i, 256)] = _tou(oTb.T)
                rel(i)
                return c

            lax.fori_loop(0, 4, phase_wo, 0)

            acq2, rel2, drain2 = stream_out(
                12, st_wqkv, lambda i: dwqkv_hbm.at[:, _ds(i, 256)], SEM_ST + 2)

            def phase_wqkv(i, c):
                acq2(i)
                st_wqkv[i % 2] = _dot(_tobf(xnT_v[...]), _tobf(dqkvT_v[_ds(i, 128), :]), NT).astype(bf)
                rel2(i)
                return c

            lax.fori_loop(0, 12, phase_wqkv, 0)

            def phase_dxa(i, c):
                rows = _ds(i, 256)
                r = _dot(wqkv_v[...], _tobf(dqkvT_v[:, rows]), NN)
                dxa_v[rows, :] = r.T
                return c

            lax.fori_loop(0, 8, phase_dxa, 0)
            drain()
            drain2()

        pl.run_scoped(post_a, pltpu.VMEM((2, 256, D), bf), pltpu.VMEM((2, D, 256), bf))

    pl.run_scoped(
        scope_a,
        pltpu.VMEM((D, 3 * D), bf),
        pltpu.VMEM((16, S // 2, 128), u32),
        pltpu.VMEM((3 * D // 2, S), u32),
        pltpu.VMEM((D // 2, S), u32),
        pltpu.VMEM((D // 2, S), u32),
        pltpu.VMEM((3 * D // 2, S), u32),
    )

    def scope_b(wsp_v, wout_v, z1_v, z2_v, gp_v, uT_v, wspT_v, rs2_v, db_v,
                st_a, st_b, st_c, st_d, st_e):
        in_copy(wsp_hbm, wsp_v, SEM_WSP).start()
        in_copy(wout_hbm, wout_v, SEM_WOUT).start()
        in_copy(win_hbm, win_v, SEM_WIN).wait()

        def phase_p1(i, c):
            ru = _ds(i, 128)
            xnb = _tobf(xn_v[ru, :])
            z2 = []
            for n in range(7):
                cs = slice(FH + n * 256, FH + (n + 1) * 256)
                z, dz = _gelu_and_grad(_dot(xnb, win_v[:, cs], NN))
                gp_v[ru, cs] = _tou(dz.astype(bf))
                z2.append(z)
            z2n, rstd = _ln_stats(jnp.concatenate(z2, axis=1))
            z2_v[ru, :] = _tou(z2n.astype(bf))
            rs2_v[_ds(i, 256), :] = jnp.broadcast_to(rstd, (256, 128))
            for n in range(7):
                cs = slice(n * 256, (n + 1) * 256)
                z, dz = _gelu_and_grad(_dot(xnb, win_v[:, cs], NN))
                gp_v[ru, cs] = _tou(dz.astype(bf))
                z1_v[ru, cs] = _tou(z.astype(bf))
            return c

        lax.fori_loop(0, 8, phase_p1, 0)

        in_copy(wsp_hbm, wsp_v, SEM_WSP).wait()
        in_copy(wout_hbm, wout_v, SEM_WOUT).wait()
        acq_o, rel_o, drain_o = stream_out(16, st_a, lambda i: out_hbm.at[_ds(i, 128)], SEM_ST)
        acq_s, rel_s, drain_s = stream_out(16, st_b, lambda i: dwsp_hbm.at[_ds(i, 128)], SEM_ST + 2)

        def phase_p2(i, c):
            acq_o(i)
            acq_s(i)
            rows = _ds(i, 128)
            ru = _ds(i, 64)
            wsp_b = wsp_v[rows, :]
            wspT_v[:, rows] = _tou(wsp_b.T)
            dout_b = dout_v[rows, :]
            bcol = jnp.broadcast_to(bsp_ref[:, rows].astype(f32), (128, 128)).T
            bcol2 = jnp.concatenate([bcol, bcol], axis=1)
            us, dgs = [], []
            dbacc = None
            for n in range(7):
                cs = slice(n * 256, (n + 1) * 256)
                g = _dot(wsp_b, _tobf(z2_v[:, cs]), NN) + bcol2
                du = _dot(dout_b, wout_v[cs, :], NT)
                z1 = _tobf(z1_v[ru, cs]).astype(f32)
                ub = (z1 * g).astype(bf)
                dg = du * z1
                part = dg[:, :128] + dg[:, 128:]
                dbacc = part if dbacc is None else dbacc + part
                dgb = dg.astype(bf)
                z1_v[ru, cs] = _tou(dgb)
                gp1 = _tobf(gp_v[ru, cs]).astype(f32)
                gp_v[ru, cs] = _tou((du * g * gp1).astype(bf))
                uT_v[n * 128:(n + 1) * 128, rows] = _tou(ub.T)
                us.append(ub)
                dgs.append(dgb)
            acc = _dot(_tobf(onat_v[ru, :]), wo_v[...], NN)
            acc = acc + _dot(jnp.concatenate(us, axis=1), wout_v[...], NN)
            st_a[i % 2] = (x_v[rows, :].astype(f32) + acc).astype(bf)
            st_b[i % 2] = _dot(jnp.concatenate(dgs, axis=1), _tobf(z2_v[...]), NT).astype(bf)
            db_v[:, rows] = jnp.sum(dbacc.T, axis=0, keepdims=True)
            rel_o(i)
            rel_s(i)
            return c

        lax.fori_loop(0, 16, phase_p2, 0)
        drain_o()
        drain_s()
        dbsp_ref[...] = db_v[...].astype(bf)

        acq_x, rel_x, drain_x = stream_out(16, st_c, lambda i: dx_hbm.at[_ds(i, 128)], SEM_ST)
        acq_w, rel_w, drain_w = stream_out(16, st_d, lambda i: dwout_hbm.at[_ds(i, 112)], SEM_ST + 2)

        def phase_p3(i, c):
            acq_x(i)
            acq_w(i)
            rows = _ds(i, 128)
            ru = _ds(i, 64)
            dy = _dot(_tobf(wspT_v[ru, :]), _tobf(z1_v[...]), NN)
            dxn = dxa_v[rows, :] + _dot(_tobf(gp_v[ru, :FH]), win_v[:, :FH], NT)
            y = _tobf(z2_v[ru, :]).astype(f32)
            rstd2 = rs2_v[rows, :][:, :1]
            dz2 = rstd2 * (dy - _rowmean(dy) - y * _rowmean(dy * y))
            dp2 = (dz2 * _tobf(gp_v[ru, FH:]).astype(f32)).astype(bf)
            gp_v[ru, FH:] = _tou(dp2)
            dxn = dxn + _dot(dp2, win_v[:, FH:], NT)
            st_d[i % 2] = _dot(_tobf(uT_v[_ds(i, 56), :]), dout_v[...], NN).astype(bf)
            xn, rstd = _ln_stats(x_v[rows, :].astype(f32))
            dx = dout_v[rows, :].astype(f32) + rstd * (dxn - _rowmean(dxn) - xn * _rowmean(dxn * xn))
            st_c[i % 2] = dx.astype(bf)
            rel_x(i)
            rel_w(i)
            return c

        lax.fori_loop(0, 16, phase_p3, 0)
        drain_x()
        drain_w()

        acq_i, rel_i, drain_i = stream_out(14, st_e, lambda i: dwin_hbm.at[:, _ds(i, 256)], SEM_ST)

        def phase_p4(i, c):
            acq_i(i)
            st_e[i % 2] = _dot(_tobf(xnT_v[...]), _tobf(gp_v[:, _ds(i, 256)]), NN).astype(bf)
            rel_i(i)
            return c

        lax.fori_loop(0, 14, phase_p4, 0)
        drain_i()

    pl.run_scoped(
        scope_b,
        pltpu.VMEM((S, S), bf),
        pltpu.VMEM((FH, D), bf),
        pltpu.VMEM((S // 2, FH), u32),
        pltpu.VMEM((S // 2, FH), u32),
        pltpu.VMEM((S // 2, F), u32),
        pltpu.VMEM((FH // 2, S), u32),
        pltpu.VMEM((S // 2, S), u32),
        pltpu.VMEM((S, 128), f32),
        pltpu.VMEM((1, S), f32),
        pltpu.VMEM((2, 128, D), bf),
        pltpu.VMEM((2, 128, S), bf),
        pltpu.VMEM((2, 128, D), bf),
        pltpu.VMEM((2, 112, D), bf),
        pltpu.VMEM((2, D, 256), bf),
    )


@jax.jit
def pallas_parallel_sum__mha_block__mixer_gmlp__prompt_kernel(
    A_x: jax.Array,
    A_wqkv: jax.Array,
    A_wo: jax.Array,
    B_x: jax.Array,
    B_w_in: jax.Array,
    B_w_sp: jax.Array,
    B_b_sp: jax.Array,
    B_w_out: jax.Array,
    grad_out: jax.Array,
):
    del B_x
    any_spec = pl.BlockSpec(memory_space=pl.ANY)
    vmem_spec = pl.BlockSpec(memory_space=pltpu.VMEM)
    out_shape = (
        jax.ShapeDtypeStruct((S, D), bf),
        jax.ShapeDtypeStruct((S, D), bf),
        jax.ShapeDtypeStruct((D, 3 * D), bf),
        jax.ShapeDtypeStruct((D, D), bf),
        jax.ShapeDtypeStruct((D, F), bf),
        jax.ShapeDtypeStruct((S, S), bf),
        jax.ShapeDtypeStruct((1, S), bf),
        jax.ShapeDtypeStruct((FH, D), bf),
    )
    outs = pl.pallas_call(
        _kernel,
        out_shape=out_shape,
        in_specs=[any_spec, any_spec, any_spec, any_spec, any_spec, vmem_spec, any_spec, any_spec],
        out_specs=(any_spec, any_spec, any_spec, any_spec, any_spec, any_spec, vmem_spec, any_spec),
        scratch_shapes=[
            pltpu.VMEM((S, D), bf),
            pltpu.VMEM((S, D), bf),
            pltpu.VMEM((D, D), bf),
            pltpu.VMEM((D, F), bf),
            pltpu.VMEM((S // 2, D), u32),
            pltpu.VMEM((D // 2, S), u32),
            pltpu.VMEM((S // 2, D), u32),
            pltpu.VMEM((S, D), f32),
            pltpu.SemaphoreType.DMA((NSEM,)),
        ],
        compiler_params=pltpu.CompilerParams(vmem_limit_bytes=127 * 1024 * 1024),
        name="mha_gmlp_fwd_bwd",
    )(
        A_x.reshape(S, D), A_wqkv, A_wo, B_w_in, B_w_sp, B_b_sp.reshape(1, S), B_w_out,
        grad_out.reshape(S, D),
    )
    out, dx, dwqkv, dwo, dwin, dwsp, dbsp, dwout = outs
    return (out.reshape(1, S, D), dx.reshape(1, S, D), dwqkv, dwo, dwin, dwsp,
            dbsp.reshape(S), dwout)
```

```python
import functools
import math

import jax
import jax.numpy as jnp
from jax import lax
import jax.experimental.pallas as pl
import jax.experimental.pallas.tpu as pltpu

S = 2048
D = 1024
H = 32
DH = 32
F = 3584
FH = F // 2
EPS = 1e-5

bf = jnp.bfloat16
f32 = jnp.float32
u32 = jnp.uint32

NN = (((1,), (0,)), ((), ()))
NT = (((1,), (1,)), ((), ()))

LN2 = math.log(2.0)
SCALE = DH ** -0.5
GELU_C = math.sqrt(2.0 / math.pi)
GELU_A = 0.044715

MQ = 512
KC = 128
NCH = S // KC
NQB = S // MQ
NBLK = H * NQB
LEAD_B = 17
LEAD_A = 36
UB = 4
QU = 2
WI = 8
P1U = 2
R2 = 128
R3 = 256
C4 = 896


def _dot(a, b, dims):
    return lax.dot_general(a, b, dims, preferred_element_type=f32)


def _tobf(x):
    return pltpu.bitcast(x, bf)


def _tou(x):
    return pltpu.bitcast(x, u32)


def _r3(x):
    return x.reshape(x.shape[0] // 8, 8, x.shape[1])


def _sub8(x, row8):
    return (_r3(x) - row8[None]).reshape(x.shape)


def _ds(i, n):
    if isinstance(i, int):
        return pl.ds(i * n, n)
    return pl.ds(pl.multiple_of(i * n, n), n)


def _rowmean(x):
    return jnp.sum(x, axis=-1, keepdims=True) * (1.0 / x.shape[-1])


def _fold128(x):
    acc = x[:, :128]
    for t in range(1, x.shape[1] // 128):
        acc = acc + x[:, t * 128:(t + 1) * 128]
    return acc


def _lanesum_b(part, scale):
    return jnp.broadcast_to(jnp.sum(part, axis=-1, keepdims=True) * scale, part.shape)


def _tile(v, w):
    return v if w == 128 else jnp.concatenate([v] * (w // 128), axis=1)


def _after(v, gate, zero):
    vi = _r3(pltpu.bitcast(v, u32))
    gi = _r3(pltpu.bitcast(gate, u32))
    return pltpu.bitcast((vi | (gi & zero[None])).reshape(v.shape), f32)


def _ln_stats(xf):
    m = _rowmean(xf)
    xc = xf - m
    v = _rowmean(xc * xc)
    rstd = lax.rsqrt(v + EPS)
    return xc * rstd, rstd


def _gelu_and_grad(x):
    u = x * x
    t = jnp.tanh(x * (GELU_C + (GELU_C * GELU_A) * u))
    h = 0.5 + 0.5 * t
    g = x * h
    dg = h + (g * (1.0 - h)) * (2.0 * GELU_C + (6.0 * GELU_C * GELU_A) * u)
    return g, dg


def _spread(tiles, nrg):
    per = [t.shape[0] // 8 for t in tiles]
    step = sum(per) / float(nrg)
    out = []
    for r in range(nrg):
        pos = int((r + 0.5) * step)
        k = 0
        while pos >= per[k]:
            pos -= per[k]
            k += 1
        out.append(tiles[k][pos * 8:(pos + 1) * 8, :])
    return jnp.concatenate(out, axis=0)


SEM_WO = 0
SEM_X = 1
SEM_DOUT = 9
SEM_WQKV = 17
SEM_WIN = 18
SEM_WSP = 19
SEM_WOUT = 20
SEM_ST = 21
SEM_W = 43
SEM_WO4 = 47
SEM_B = 51
NSEM = 52


def _kernel(x_hbm, wqkv_hbm, wo_hbm, win_hbm, wsp_hbm, bsp_hbm, wout_hbm, dout_hbm,
            out_hbm, dx_hbm, dwqkv_hbm, dwo_hbm, dwin_hbm, dwsp_hbm, dbsp_hbm, dwout_hbm,
            x_v, dout_v, wo_v, win_v, xn_v, xnT_v, onat_v, dxa_v, rsx_v, zero_v, st_wo, st_wqkv, sems):

    zero_v[...] = jnp.zeros_like(zero_v)

    def in_copy(src, dst, s):
        return pltpu.make_async_copy(src, dst, sems.at[s])

    def x_copy(i):
        return in_copy(x_hbm.at[_ds(i, 256)], x_v.at[_ds(i, 256)], SEM_X + i)

    def dout_copy(i):
        return in_copy(dout_hbm.at[_ds(i, 256)], dout_v.at[_ds(i, 256)], SEM_DOUT + i)

    def stream_out(n_iters, stage, dst_fn, sem0):
        def cp(i, slot):
            return pltpu.make_async_copy(stage.at[slot], dst_fn(i), sems.at[sem0 + slot])

        def acquire(i):
            @pl.when(i >= 2)
            def _():
                cp(i - 2, i % 2).wait()

        def release(i):
            cp(i, i % 2).start()

        def drain():
            cp(n_iters - 2, n_iters % 2).wait()
            cp(n_iters - 1, (n_iters - 1) % 2).wait()

        return acquire, release, drain

    ro = D // WI
    cq = 3 * D // WI
    rt = S // WI
    acq_wo, rel_wo, drain_wo = stream_out(WI, st_wo, lambda i: dwo_hbm.at[_ds(i, ro)], SEM_W)
    acq_wq, rel_wq, drain_wq = stream_out(WI, st_wqkv, lambda i: dwqkv_hbm.at[:, _ds(i, cq)], SEM_W + 2)

    def scope_a(wqkv_v, kv_v, qkvT_v, dOT_v, oT_v, dqkvT_v):
        def wo_copy(k):
            return in_copy(wo_hbm.at[pl.ds(k * 256, 256)], wo_v.at[pl.ds(k * 256, 256)], SEM_WO4 + k)

        dout_copy(0).start()
        wo_copy(0).start()
        x_copy(0).start()
        for k in range(1, 4):
            wo_copy(k).start()
        for i in range(1, 8):
            dout_copy(i).start()
            x_copy(i).start()
        in_copy(wqkv_hbm, wqkv_v, SEM_WQKV).start()

        def phase_d(i, c):
            first = isinstance(i, int)
            dout_copy(i).wait()
            if not first:
                x_copy(i).wait()
            rows = _ds(i, 256)
            zero = zero_v[:, :128]
            dout_b = dout_v[rows, :]
            gates = []
            for k in range(4):
                if first:
                    wo_copy(k).wait()
                    if k == 1:
                        x_copy(i).wait()
                dot_b = _dot(wo_v[k * 256:(k + 1) * 256, :], dout_b, NT)
                dOT_v[k * 128:(k + 1) * 128, rows] = _tou(dot_b.astype(bf))
                gates += [dot_b[:, :128], dot_b[:, 128:]]
            tiles = [slice(t * 128, (t + 1) * 128) for t in range(D // 128)]
            s1 = _fold128(x_v[rows, :].astype(f32))
            m = _after(_lanesum_b(s1, 1.0 / D), _spread(gates[0:3], 32), zero)
            s2 = None
            for ts in tiles:
                xc = x_v[rows, ts].astype(f32) - m
                s2 = xc * xc if s2 is None else s2 + xc * xc
            rstd = lax.rsqrt(_lanesum_b(s2, 1.0 / D) + EPS)
            rsx_v[rows, :] = rstd
            rstd = _after(rstd, _spread(gates[4:6], 32), zero)
            mr = m * rstd
            xnb = jnp.concatenate(
                [(x_v[rows, ts].astype(f32) * rstd - mr).astype(bf) for ts in tiles], axis=1)
            xn_v[_ds(i, 128), :] = _tou(xnb)
            xnT_v[:, rows] = _tou(xnb.T)
            return c

        phase_d(0, 0)
        lax.fori_loop(1, 8, phase_d, 0)

        in_copy(win_hbm, win_v, SEM_WIN).start()
        in_copy(wqkv_hbm, wqkv_v, SEM_WQKV).wait()

        def phase_q(ii, c):
            for sub in range(QU):
                i = ii * QU + sub
                rows = _ds(i, 256)
                xnb = _tobf(xn_v[_ds(i, 128), :])
                chunks = [(1024, 512), (1536, 512), (2048, 512), (2560, 512), (0, 512), (512, 256),
                          (768, 128), (896, 128)]
                for c0, w in chunks:
                    r = _dot(xnb, wqkv_v[:, c0:c0 + w], NN)
                    if c0 < D:
                        r = r * (SCALE / LN2)
                    rb = r.astype(bf)
                    if c0 >= D:
                        ru = _tou(rb)
                        for p in range(w // 128):
                            kv_v[(c0 - D) // 128 + p, _ds(i, 128), :] = ru[:, p * 128:(p + 1) * 128]
                    qkvT_v[c0 // 2:(c0 + w) // 2, rows] = _tou(rb.T)
            return c

        lax.fori_loop(0, 8 // QU, phase_q, 0)

        def attention(s_buf0, s_buf1, p_buf0, p_buf1, m_buf, dos_buf, dl_buf, dk_acc, dv_acc, ds_buf):
            for r in (dk_acc, dv_acc, ds_buf):
                r[...] = jnp.zeros_like(r)
            s_bufs = (s_buf0, s_buf1)
            p_bufs = (p_buf0, p_buf1)
            lane_h = lax.broadcasted_iota(jnp.int32, (64, 128), 1) // 32

            def bc8(v):
                return jnp.broadcast_to(v, (8, MQ))

            def blk(b, rel):
                if isinstance(b, int):
                    b = min(max(b, 0), NBLK - 1)
                    h = b // NQB
                    qb = b % NQB
                    return dict(g=h // 4, r=h % 4, q=pl.ds(qb * MQ, MQ), s=rel % 2,
                                g64=pl.ds((h // 4) * 64, 64),
                                row=lambda base: pl.ds(base + h * 16, 16),
                                first=(qb == 0), last=(qb == NQB - 1), cache={})
                h = jnp.clip(b, 0, NBLK - 1) // NQB
                if UB % NQB == 0:
                    qb = rel % NQB
                    q, first, last = pl.ds(qb * MQ, MQ), qb == 0, qb == NQB - 1
                else:
                    qb = jnp.clip(b, 0, NBLK - 1) % NQB
                    q = pl.ds(pl.multiple_of(qb * MQ, MQ), MQ)
                    first, last = (qb == 0) if rel % 2 == 0 else False, rel % 2 == 1
                return dict(g=h // 4, r=h % 4, q=q, s=rel % 2,
                            g64=pl.ds(pl.multiple_of((h // 4) * 64, 64), 64),
                            row=lambda base: pl.ds(pl.multiple_of(base + h * 16, 16), 16),
                            first=first, last=last, cache={})

            def accum(first, acc_ref, ks, new):
                if first is True:
                    return new
                old = acc_ref[:, ks]
                if first is not False:
                    old = jnp.where(first, 0.0, old)
                return old + new

            def steps(get_blk, tau0, n, st, pos_max):
                def do_dkdq(c, j, dsb):
                    ks = slice(j * KC, (j + 1) * KC)
                    if 'qT' not in c['cache']:
                        c['cache']['qT'] = _tobf(qkvT_v[c['row'](0), c['q']])
                    dk_new = accum(c['first'], dk_acc, ks, _dot(c['cache']['qT'], dsb, NT))
                    if not (c['last'] and UB % NQB == 0):
                        dk_acc[:, ks] = dk_new
                    if c['last']:
                        dqkvT_v[c['row'](512), ks] = _tou((dk_new * LN2).astype(bf))
                    kT = _tobf(qkvT_v[c['row'](512), ks])
                    dq = _dot(kT, dsb, NN)
                    st['dq'] = dq if j == 0 else st['dq'] + dq
                    if j == NCH - 1:
                        dqkvT_v[c['row'](0), c['q']] = _tou((st['dq'] * SCALE).astype(bf))

                for tau in range(tau0, tau0 + n):
                    pos_b = tau + LEAD_B
                    do_b = 0 <= pos_b < pos_max
                    if do_b:
                        b = get_blk(pos_b // NCH)
                        jb = pos_b % NCH
                        mb = m_buf[b['s']]
                        if st['cm'] is not None:
                            mb = _after(mb, st['cm'], zero_v[...])
                        p = jnp.exp2(_sub8(s_bufs[b['s']][jb * KC:(jb + 1) * KC, :], mb))
                        acc = p[KC - 8:KC] if jb == 0 else st['l'] + p[KC - 8:KC]
                        for i in range(KC // 8 - 2, -1, -1):
                            acc = acc + p[i * 8:(i + 1) * 8]
                        st['l'] = acc
                        pbn = p.astype(bf)
                        p_bufs[b['s']][jb * 64:(jb + 1) * 64, :] = _tou(pbn)
                    if tau >= 0:
                        c = get_blk(tau // NCH)
                        j = tau % NCH
                        ks = slice(j * KC, (j + 1) * KC)
                        ksu = slice(j * 64, (j + 1) * 64)
                        if 'dosT' not in c['cache']:
                            c['cache']['dosT'] = _tobf(dos_buf[c['s']])
                            c['cache']['dos4'] = jnp.concatenate([c['cache']['dosT']] * 4, axis=0)
                            c['cache']['dl'] = dl_buf[c['s']]
                        v4 = _tobf(jnp.where(lane_h == c['r'], kv_v[8 + c['g'], ksu, :], jnp.uint32(0)))
                        dpT = _dot(v4, c['cache']['dos4'], NN)
                        pb = _tobf(p_bufs[c['s']][ksu, :])
                        dv_new = accum(c['first'], dv_acc, ks, _dot(c['cache']['dosT'], pb, NT))
                        if not (c['last'] and UB % NQB == 0):
                            dv_acc[:, ks] = dv_new
                        if c['last']:
                            dqkvT_v[c['row'](1024), ks] = _tou(dv_new.astype(bf))
                        dsb = (pb.astype(f32) * _sub8(dpT, c['cache']['dl'])).astype(bf)
                        if st['pend'] is not None:
                            do_dkdq(*st['pend'])
                        st['pend'] = (c, j, dsb)
                    pos_a = tau + LEAD_A
                    if pos_a < pos_max:
                        a = get_blk(pos_a // NCH)
                        ja = pos_a % NCH
                        kau = slice(ja * 64, (ja + 1) * 64)
                        k4 = _tobf(jnp.where(lane_h == a['r'], kv_v[a['g'], kau, :], jnp.uint32(0)))
                        sT = _dot(k4, _tobf(qkvT_v[a['g64'], a['q']]), NN)
                        s_bufs[a['s']][ja * KC:(ja + 1) * KC, :] = sT
                        cm = jnp.max(_r3(sT), axis=0)
                        st['cm'] = cm
                        st['m'] = cm if ja == 0 else jnp.maximum(st['m'], cm)
                        if ja == NCH - 1:
                            m_buf[a['s']] = bc8(jnp.max(st['m'], axis=0, keepdims=True))
                    else:
                        st['cm'] = dpT[0:8]
                    if do_b:
                        vT = _tobf(qkvT_v[b['row'](1024), jb * KC:(jb + 1) * KC])
                        o = _dot(vT, pbn, NN)
                        st['ot'] = o if jb == 0 else st['ot'] + o
                        if jb == NCH - 1:
                            rl = 1.0 / jnp.sum(st['l'], axis=0, keepdims=True)
                            ot = st['ot'] * rl
                            oT_v[b['row'](0), b['q']] = _tou(ot.astype(bf))
                            dob = _tobf(dOT_v[b['row'](0), b['q']]).astype(f32) * rl
                            dos_buf[b['s']] = _tou(dob.astype(bf))
                            dl_buf[b['s']] = bc8(jnp.sum(dob * ot, axis=0, keepdims=True))
                return do_dkdq

            def blk_getter(base):
                cache = {}

                def get(rb):
                    if rb not in cache:
                        cache[rb] = blk(base + rb, rb)
                    return cache[rb]

                return get

            nstep = UB * NCH
            nit = NBLK // UB - 1
            big = 1 << 30
            st = dict(m=None, l=None, ot=None, dq=None, pend=None, cm=None)
            steps(blk_getter(0), -LEAD_A, LEAD_A, st, big)

            def body(it, carry):
                m, l, ot, dq = carry
                get = blk_getter(it * UB)
                st = dict(m=m, l=l, ot=ot, dq=dq, cm=None, pend=(get(-1), NCH - 1, _tobf(ds_buf[...])))
                steps(get, 0, nstep, st, big)
                ds_buf[...] = _tou(st['pend'][2])
                return st['m'], st['l'], st['ot'], st['dq']

            m, l, ot, dq = lax.fori_loop(
                0, nit, body, (st['m'], st['l'], st['ot'], jnp.zeros((32, MQ), f32)))
            get = blk_getter(0)
            t0 = nit * nstep
            st = dict(m=m, l=l, ot=ot, dq=dq, cm=None,
                      pend=(get(t0 // NCH - 1), NCH - 1, _tobf(ds_buf[...])))
            fin = steps(get, t0, nstep, st, NBLK * NCH)
            fin(*st['pend'])

        pl.run_scoped(
            attention,
            pltpu.VMEM((S, MQ), f32), pltpu.VMEM((S, MQ), f32),
            pltpu.VMEM((S // 2, MQ), u32), pltpu.VMEM((S // 2, MQ), u32),
            pltpu.VMEM((2, 8, MQ), f32), pltpu.VMEM((2, 16, MQ), u32), pltpu.VMEM((2, 8, MQ), f32),
            pltpu.VMEM((32, S), f32), pltpu.VMEM((32, S), f32), pltpu.VMEM((64, MQ), u32),
        )

        if True:
            acq, rel = acq_wo, rel_wo
            acq2, rel2 = acq_wq, rel_wq

            def phase_w(i, c):
                acq(i)
                acq2(i)
                for k in range(rt // 256):
                    rows = pl.ds(pl.multiple_of(i * rt + k * 256, 256), 256)
                    dq_b = _tobf(dqkvT_v[:, rows])
                    for m in range(4):
                        r = _dot(wqkv_v[m * 256:(m + 1) * 256, :], dq_b, NN)
                        dxa_v[rows, m * 256:(m + 1) * 256] = r.T
                oTb = _tobf(oT_v[_ds(i, ro // 2), :])
                onat_v[:, _ds(i, ro)] = _tou(oTb.T)
                st_wo[i % 2] = _dot(oTb, dout_v[...], NN).astype(bf)
                rel(i)
                st_wqkv[i % 2] = _dot(_tobf(xnT_v[...]), _tobf(dqkvT_v[_ds(i, cq // 2), :]), NT).astype(bf)
                rel2(i)
                return c

            lax.fori_loop(0, WI, phase_w, 0)

    pl.run_scoped(
        scope_a,
        pltpu.VMEM((D, 3 * D), bf),
        pltpu.VMEM((16, S // 2, 128), u32),
        pltpu.VMEM((3 * D // 2, S), u32),
        pltpu.VMEM((D // 2, S), u32),
        pltpu.VMEM((D // 2, S), u32),
        pltpu.VMEM((3 * D // 2, S), u32),
    )

    def scope_b(wsp_v, wout_v, z1_v, z2_v, gp_v, uT_v, wspT_v, rs2_v, db_v, bs_v, zf_v,
                st_a, st_b, st_c, st_d, st_e):
        in_copy(wsp_hbm, wsp_v, SEM_WSP).start()
        in_copy(wout_hbm, wout_v, SEM_WOUT).start()
        in_copy(bsp_hbm, bs_v.at[pl.ds(0, 16)], SEM_B).start()
        in_copy(win_hbm, win_v, SEM_WIN).wait()

        def phase_p1(ii, c):
            for sub in range(P1U):
                i = ii * P1U + sub
                ru = _ds(i, 128)
                xnb = _tobf(xn_v[ru, :])
                zf = zf_v.at[sub]
                s1 = None
                for n in range(7):
                    cs = slice(FH + n * 256, FH + (n + 1) * 256)
                    z, dz = _gelu_and_grad(_dot(xnb, win_v[:, cs], NN))
                    gp_v[ru, cs] = _tou(dz.astype(bf))
                    zf[:, n * 256:(n + 1) * 256] = z
                    s1 = _fold128(z) if s1 is None else s1 + _fold128(z)
                gates = []
                for c0, w in [(n * 256, 256) for n in range(6)] + [(1536, 128), (1664, 128)]:
                    cs = slice(c0, c0 + w)
                    pre = _dot(xnb, win_v[:, cs], NN)
                    gates += [pre[:, t * 128:(t + 1) * 128] for t in range(w // 128)]
                    z, dz = _gelu_and_grad(pre)
                    gp_v[ru, cs] = _tou(dz.astype(bf))
                    z1_v[ru, cs] = _tou(z.astype(bf))
                zero = zero_v[:, :128]
                m = _after(_lanesum_b(s1, 1.0 / FH), _spread(gates[1:7], 32), zero)
                s2 = None
                for t in range(FH // 128):
                    zc = zf[:, t * 128:(t + 1) * 128] - m
                    s2 = zc * zc if s2 is None else s2 + zc * zc
                rstd = lax.rsqrt(_lanesum_b(s2, 1.0 / FH) + EPS)
                rs2_v[_ds(i, 256), :] = rstd
                rstd = _after(rstd, _spread(gates[8:13], 32), zero)
                mr = m * rstd
                for t in range(FH // 128):
                    ts = slice(t * 128, (t + 1) * 128)
                    z2_v[ru, ts] = _tou((zf[:, ts] * rstd - mr).astype(bf))
            return c

        lax.fori_loop(0, 8 // P1U, phase_p1, 0)

        in_copy(wsp_hbm, wsp_v, SEM_WSP).wait()
        in_copy(wout_hbm, wout_v, SEM_WOUT).wait()
        n2 = S // R2
        in_copy(bsp_hbm, bs_v.at[pl.ds(0, 16)], SEM_B).wait()
        db_v[0:16, :] = bs_v[0:16, :].astype(f32)
        acq_o, rel_o, drain_o = stream_out(n2, st_a, lambda i: out_hbm.at[_ds(i, R2)], SEM_ST)
        acq_s, rel_s, drain_s = stream_out(n2, st_b, lambda i: dwsp_hbm.at[_ds(i, R2)], SEM_ST + 2)

        def phase_p2(i, c):
            acq_o(i)
            acq_s(i)
            rows = _ds(i, R2)
            ru = _ds(i, R2 // 2)
            wsp_b = wsp_v[rows, :]
            wspT_v[:, rows] = _tou(wsp_b.T)
            dout_b = dout_v[rows, :]
            bcol = jnp.broadcast_to(db_v[pl.ds(i, 1), :], (128, 128)).T
            bcol2 = jnp.concatenate([bcol, bcol], axis=1)
            us, dgs = [], []
            dbacc = None
            for n in range(7):
                cs = slice(n * 256, (n + 1) * 256)
                g = _dot(wsp_b, _tobf(z2_v[:, cs]), NN) + bcol2
                du = _dot(dout_b, wout_v[cs, :], NT)
                z1 = _tobf(z1_v[ru, cs]).astype(f32)
                ub = (z1 * g).astype(bf)
                dg = du * z1
                part = dg[:, :128] + dg[:, 128:]
                dbacc = part if dbacc is None else dbacc + part
                dgb = dg.astype(bf)
                z1_v[ru, cs] = _tou(dgb)
                gp1 = _tobf(gp_v[ru, cs]).astype(f32)
                gp_v[ru, cs] = _tou((du * g * gp1).astype(bf))
                uT_v[n * 128:(n + 1) * 128, rows] = _tou(ub.T)
                us.append(ub)
                dgs.append(dgb)
            acc = _dot(_tobf(onat_v[ru, :]), wo_v[...], NN)
            acc = acc + _dot(jnp.concatenate(us, axis=1), wout_v[...], NN)
            st_a[i % 2] = (x_v[rows, :].astype(f32) + acc).astype(bf)
            rel_o(i)
            db_v[pl.ds(i, 1), :] = jnp.sum(dbacc.T, axis=0, keepdims=True)
            st_b[i % 2] = _dot(jnp.concatenate(dgs, axis=1), _tobf(z2_v[...]), NT).astype(bf)
            rel_s(i)
            return c

        lax.fori_loop(0, n2, phase_p2, 0)
        bs_v[0:16, :] = db_v[0:16, :].astype(bf)
        in_copy(bs_v.at[pl.ds(0, 16)], dbsp_hbm, SEM_B).start()

        n3 = S // R3
        rw = FH // n3
        acq_x, rel_x, drain_x = stream_out(n3, st_c, lambda i: dx_hbm.at[_ds(i, R3)], SEM_ST + 4)
        acq_w, rel_w, drain_w = stream_out(n3, st_d, lambda i: dwout_hbm.at[_ds(i, rw)], SEM_ST + 6)

        def phase_p3(i, c):
            acq_x(i)
            acq_w(i)
            rows = _ds(i, R3)
            ru = _ds(i, R3 // 2)
            wb = _tobf(wspT_v[ru, :])
            dyf = zf_v.at[0, :R3]
            sa = sb = None
            for n in range(7):
                cs = slice(n * 256, (n + 1) * 256)
                dy = _dot(wb, _tobf(z1_v[:, cs]), NN)
                dyf[:, cs] = dy
                pa = _fold128(dy)
                pb = _fold128(dy * _tobf(z2_v[ru, cs]).astype(f32))
                sa = pa if sa is None else sa + pa
                sb = pb if sb is None else sb + pb
            zero = zero_v[:, :128]
            dp1 = _tobf(gp_v[ru, :FH])
            dxn1 = [_dot(dp1, win_v[n * 256:(n + 1) * 256, :FH], NT) for n in range(4)]
            rstd2 = rs2_v[rows, :]
            gate = _spread([d[:, t * 128:(t + 1) * 128] for d in dxn1[:3] for t in range(2)], R3 // 8)
            ra = _after(_lanesum_b(sa, 1.0 / FH), gate, zero)
            rb = _after(_lanesum_b(sb, 1.0 / FH), gate, zero)
            dp2 = []
            for t in range(FH // 128):
                ts = slice(t * 128, (t + 1) * 128)
                gs = slice(FH + t * 128, FH + (t + 1) * 128)
                dz2 = ((dyf[:, ts] - ra) - _tobf(z2_v[ru, ts]).astype(f32) * rb) * rstd2
                d = (dz2 * _tobf(gp_v[ru, gs]).astype(f32)).astype(bf)
                gp_v[ru, gs] = _tou(d)
                dp2.append(d)
            dp2 = jnp.concatenate(dp2, axis=1)
            dxf = zf_v.at[1, :R3]
            sa = sb = None
            for n in range(4):
                cs = slice(n * 256, (n + 1) * 256)
                dxn = (dxa_v[rows, cs] + dxn1[n]) + _dot(dp2, win_v[cs, FH:], NT)
                dxf[:, cs] = dxn
                pa = _fold128(dxn)
                pb = _fold128(dxn * _tobf(xn_v[ru, cs]).astype(f32))
                sa = pa if sa is None else sa + pa
                sb = pb if sb is None else sb + pb
            uTb = _tobf(uT_v[_ds(i, rw // 2), :])
            dwo = [_dot(uTb, dout_v[:, n * 256:(n + 1) * 256], NN) for n in range(4)]
            for n in range(4):
                st_d[i % 2, :, n * 256:(n + 1) * 256] = dwo[n].astype(bf)
            gate = _spread([d[:, t * 128:(t + 1) * 128] for d in dwo[:3] for t in range(2)], R3 // 8)
            rstd = rsx_v[rows, :]
            ra = _after(_lanesum_b(sa, 1.0 / D), gate, zero)
            rb = _after(_lanesum_b(sb, 1.0 / D), gate, zero)
            for t in range(D // 128):
                ts = slice(t * 128, (t + 1) * 128)
                dx = (((dxf[:, ts] - ra) - _tobf(xn_v[ru, ts]).astype(f32) * rb) * rstd
                      + dout_v[rows, ts].astype(f32))
                st_c[i % 2, :, ts] = dx.astype(bf)
            rel_x(i)
            rel_w(i)
            return c

        lax.fori_loop(0, n3, phase_p3, 0)

        n4 = F // C4
        np4 = C4 // 128

        def cp4(i, k):
            return pltpu.make_async_copy(
                st_e.at[i % 2, k], dwin_hbm.at[:, pl.ds(pl.multiple_of(i * C4 + k * 128, 128), 128)],
                sems.at[SEM_ST + 8 + (i % 2) * np4 + k])

        def drain_i():
            for i in (n4 - 2, n4 - 1):
                for k in range(np4):
                    cp4(i, k).wait()

        def phase_p4(i, c):
            @pl.when(i >= 2)
            def _():
                for k in range(np4):
                    cp4(i - 2, k).wait()

            xnT = _tobf(xnT_v[...])
            for k in range(np4):
                cols = pl.ds(pl.multiple_of(i * C4 + k * 128, 128), 128)
                st_e[i % 2, k] = _dot(xnT, _tobf(gp_v[:, cols]), NN).astype(bf)
                cp4(i, k).start()
            return c

        lax.fori_loop(0, n4, phase_p4, 0)
        in_copy(bs_v.at[pl.ds(0, 16)], dbsp_hbm, SEM_B).wait()
        drain_wo()
        drain_wq()
        drain_o()
        drain_s()
        drain_x()
        drain_w()
        drain_i()

    pl.run_scoped(
        scope_b,
        pltpu.VMEM((S, S), bf),
        pltpu.VMEM((FH, D), bf),
        pltpu.VMEM((S // 2, FH), u32),
        pltpu.VMEM((S // 2, FH), u32),
        pltpu.VMEM((S // 2, F), u32),
        pltpu.VMEM((FH // 2, S), u32),
        pltpu.VMEM((S // 2, S), u32),
        pltpu.VMEM((S, 128), f32),
        pltpu.VMEM((32, 128), f32),
        pltpu.VMEM((64, 128), bf),
        pltpu.VMEM((2, 256, FH), f32),
        pltpu.VMEM((2, R2, D), bf),
        pltpu.VMEM((2, R2, S), bf),
        pltpu.VMEM((2, R3, D), bf),
        pltpu.VMEM((2, FH * R3 // S, D), bf),
        pltpu.VMEM((2, C4 // 128, D, 128), bf),
    )


@jax.jit
def pallas_parallel_sum__mha_block__mixer_gmlp__prompt_kernel(
    A_x: jax.Array,
    A_wqkv: jax.Array,
    A_wo: jax.Array,
    B_x: jax.Array,
    B_w_in: jax.Array,
    B_w_sp: jax.Array,
    B_b_sp: jax.Array,
    B_w_out: jax.Array,
    grad_out: jax.Array,
):
    del B_x
    any_spec = pl.BlockSpec(memory_space=pl.ANY)
    vmem_spec = pl.BlockSpec(memory_space=pltpu.VMEM)
    out_shape = (
        jax.ShapeDtypeStruct((S, D), bf),
        jax.ShapeDtypeStruct((S, D), bf),
        jax.ShapeDtypeStruct((D, 3 * D), bf),
        jax.ShapeDtypeStruct((D, D), bf),
        jax.ShapeDtypeStruct((D, F), bf),
        jax.ShapeDtypeStruct((S, S), bf),
        jax.ShapeDtypeStruct((S // 128, 128), bf),
        jax.ShapeDtypeStruct((FH, D), bf),
    )
    outs = pl.pallas_call(
        _kernel,
        out_shape=out_shape,
        in_specs=[any_spec] * 8,
        out_specs=(any_spec,) * 8,
        scratch_shapes=[
            pltpu.VMEM((S, D), bf),
            pltpu.VMEM((S, D), bf),
            pltpu.VMEM((D, D), bf),
            pltpu.VMEM((D, F), bf),
            pltpu.VMEM((S // 2, D), u32),
            pltpu.VMEM((D // 2, S), u32),
            pltpu.VMEM((S // 2, D), u32),
            pltpu.VMEM((S, D), f32),
            pltpu.VMEM((S, 128), f32),
            pltpu.VMEM((8, MQ), u32),
            pltpu.VMEM((2, D // WI, D), bf),
            pltpu.VMEM((2, D, 3 * D // WI), bf),
            pltpu.SemaphoreType.DMA((NSEM,)),
        ],
        compiler_params=pltpu.CompilerParams(vmem_limit_bytes=127 * 1024 * 1024),
        name="mha_gmlp_fwd_bwd",
    )(
        A_x.reshape(S, D), A_wqkv, A_wo, B_w_in, B_w_sp, B_b_sp.reshape(S // 128, 128), B_w_out,
        grad_out.reshape(S, D),
    )
    out, dx, dwqkv, dwo, dwin, dwsp, dbsp, dwout = outs
    return (out.reshape(1, S, D), dx.reshape(1, S, D), dwqkv, dwo, dwin, dwsp,
            dbsp.reshape(S), dwout)
```

```python
import math

import jax
import jax.numpy as jnp
from jax import lax
import jax.experimental.pallas as pl
import jax.experimental.pallas.tpu as pltpu

S = 2048
D = 1024
H = 32
DH = 32
F = 3584
FH = F // 2
EPS = 1e-5

bf = jnp.bfloat16
f32 = jnp.float32
u32 = jnp.uint32

NN = (((1,), (0,)), ((), ()))
NT = (((1,), (1,)), ((), ()))

LN2 = math.log(2.0)
SCALE = DH ** -0.5
GELU_C = math.sqrt(2.0 / math.pi)
GELU_A = 0.044715

MQ = 512
KC = 128
NCH = S // KC
NQB = S // MQ
NBLK = H * NQB
LEAD_B = 17
LEAD_A = 36
UB = NQB

QU = 2
WI = 8
P1U = 2
R2 = 256
R3 = 256
C4 = 896


def _dot(a, b, dims):
    return lax.dot_general(a, b, dims, preferred_element_type=f32)


def _tobf(x):
    return pltpu.bitcast(x, bf)


def _tou(x):
    return pltpu.bitcast(x, u32)


def _r3(x):
    return x.reshape(x.shape[0] // 8, 8, x.shape[1])


def _sub8(x, row8):
    return (_r3(x) - row8[None]).reshape(x.shape)


def _ds(i, n):
    if isinstance(i, int):
        return pl.ds(i * n, n)
    return pl.ds(pl.multiple_of(i * n, n), n)


def _fold128(x):
    acc = x[:, :128]
    for t in range(1, x.shape[1] // 128):
        acc = acc + x[:, t * 128:(t + 1) * 128]
    return acc


def _lanesum_b(part, scale):
    return jnp.broadcast_to(jnp.sum(part, axis=-1, keepdims=True) * scale, part.shape)


def _after(v, gate, zero):
    vi = _r3(pltpu.bitcast(v, u32))
    gi = _r3(pltpu.bitcast(gate, u32))
    return pltpu.bitcast((vi | (gi & zero[None])).reshape(v.shape), f32)


def _gelu_and_grad(x):
    u = x * x
    t = jnp.tanh(x * (GELU_C + (GELU_C * GELU_A) * u))
    h = 0.5 + 0.5 * t
    g = x * h
    dg = h + (g * (1.0 - h)) * (2.0 * GELU_C + (6.0 * GELU_C * GELU_A) * u)
    return g, dg


def _spread(tiles, nrg):
    per = [t.shape[0] // 8 for t in tiles]
    step = sum(per) / float(nrg)
    out = []
    for r in range(nrg):
        pos = int((r + 0.5) * step)
        k = 0
        while pos >= per[k]:
            pos -= per[k]
            k += 1
        out.append(tiles[k][pos * 8:(pos + 1) * 8, :])
    return jnp.concatenate(out, axis=0)


SEM_X = 1
SEM_DOUT = 9
SEM_WQKV = 17
SEM_WIN = 18
SEM_WSP = 19
SEM_WOUT = 20
SEM_ST = 21
SEM_W = 43
SEM_WO4 = 47
SEM_B = 51
NSEM = 52


def _kernel(x_hbm, wqkv_hbm, wo_hbm, win_hbm, wsp_hbm, bsp_hbm, wout_hbm, dout_hbm,
            out_hbm, dx_hbm, dwqkv_hbm, dwo_hbm, dwin_hbm, dwsp_hbm, dbsp_hbm, dwout_hbm,
            x_v, dout_v, wo_v, win_v, xn_v, xnT_v, onat_v, dxa_v, rsx_v, zero_v, st_wo, st_wqkv, sems):

    zero_v[...] = jnp.zeros_like(zero_v)

    def in_copy(src, dst, s):
        return pltpu.make_async_copy(src, dst, sems.at[s])

    def x_copy(i):
        return in_copy(x_hbm.at[_ds(i, 256)], x_v.at[_ds(i, 256)], SEM_X + i)

    def dout_copy(i):
        return in_copy(dout_hbm.at[_ds(i, 256)], dout_v.at[_ds(i, 256)], SEM_DOUT + i)

    def stream_out(n_iters, stage, dst_fn, sem0):
        def cp(i, slot):
            return pltpu.make_async_copy(stage.at[slot], dst_fn(i), sems.at[sem0 + slot])

        def acquire(i):
            @pl.when(i >= 2)
            def _():
                cp(i - 2, i % 2).wait()

        def release(i):
            cp(i, i % 2).start()

        def drain():
            cp(n_iters - 2, n_iters % 2).wait()
            cp(n_iters - 1, (n_iters - 1) % 2).wait()

        return acquire, release, drain

    ro = D // WI
    cq = 3 * D // WI
    rt = S // WI
    acq_wo, rel_wo, drain_wo = stream_out(WI, st_wo, lambda i: dwo_hbm.at[_ds(i, ro)], SEM_W)
    acq_wq, rel_wq, drain_wq = stream_out(WI, st_wqkv, lambda i: dwqkv_hbm.at[:, _ds(i, cq)], SEM_W + 2)

    def scope_a(wqkv_v, kv_v, qkvT_v, dOT_v, oT_v, dqkvT_v):
        def wo_copy(k):
            return in_copy(wo_hbm.at[pl.ds(k * 256, 256)], wo_v.at[pl.ds(k * 256, 256)], SEM_WO4 + k)

        dout_copy(0).start()
        wo_copy(0).start()
        wo_copy(1).start()
        dout_copy(1).start()
        wo_copy(2).start()
        wo_copy(3).start()
        for i in range(2, 8):
            x_copy(i - 2).start()
            dout_copy(i).start()
        x_copy(6).start()
        x_copy(7).start()
        in_copy(wqkv_hbm, wqkv_v, SEM_WQKV).start()

        def do_dot(i, k):
            rows = _ds(i, 256)
            dot_b = _dot(wo_v[k * 256:(k + 1) * 256, :], dout_v[rows, :], NT)
            dOT_v[k * 128:(k + 1) * 128, rows] = _tou(dot_b.astype(bf))
            return [dot_b[:, :128], dot_b[:, 128:]]

        def do_ln(i, gates):
            rows = _ds(i, 256)
            zero = zero_v[:, :128]
            tiles = [slice(t * 128, (t + 1) * 128) for t in range(D // 128)]
            s1 = _fold128(x_v[rows, :].astype(f32))
            m = _after(_lanesum_b(s1, 1.0 / D), _spread(gates[0:3], 32), zero)
            s2 = None
            for ts in tiles:
                xc = x_v[rows, ts].astype(f32) - m
                s2 = xc * xc if s2 is None else s2 + xc * xc
            rstd = lax.rsqrt(_lanesum_b(s2, 1.0 / D) + EPS)
            rsx_v[rows, :] = rstd
            rstd = _after(rstd, _spread(gates[4:6], 32), zero)
            mr = m * rstd
            xnb = jnp.concatenate(
                [(x_v[rows, ts].astype(f32) * rstd - mr).astype(bf) for ts in tiles], axis=1)
            xn_v[_ds(i, 128), :] = _tou(xnb)
            xnT_v[:, rows] = _tou(xnb.T)

        def phase_d0():
            dout_copy(0).wait()
            wo_copy(0).wait()
            do_dot(0, 0)
            wo_copy(1).wait()
            do_dot(0, 1)
            dout_copy(1).wait()
            do_dot(1, 0)
            do_dot(1, 1)
            wo_copy(2).wait()
            do_dot(0, 2)
            do_dot(1, 2)
            wo_copy(3).wait()
            do_dot(0, 3)
            do_dot(1, 3)

        def phase_d(i, c):
            x_copy(i - 2).wait()
            dout_copy(i).wait()
            gates = []
            for k in range(4):
                gates += do_dot(i, k)
            do_ln(i - 2, gates)
            return c

        phase_d0()
        lax.fori_loop(2, 8, phase_d, 0)

        in_copy(win_hbm, win_v, SEM_WIN).start()
        in_copy(wqkv_hbm, wqkv_v, SEM_WQKV).wait()

        x_copy(6).wait()
        x_copy(7).wait()

        def late_vt(i):
            qkvT_v[3 * D // 2 - 64:, _ds(i, 256)] = _tou(_tobf(kv_v[15, _ds(i, 128), :]).T)

        def phase_q(ii, c):
            qgates = []
            if not isinstance(ii, int):
                late_vt(ii * QU - 1)
            for sub in range(QU):
                i = ii * QU + sub
                rows = _ds(i, 256)
                xnb = _tobf(xn_v[_ds(i, 128), :])
                chunks = [(0, 512), (512, 512), (1024, 512), (1536, 512), (2048, 512), (2560, 384),
                          (2944, 128)]
                for c0, w in chunks:
                    r = _dot(xnb, wqkv_v[:, c0:c0 + w], NN)
                    qgates += [r[:, t * 128:(t + 1) * 128] for t in range(w // 128)]
                    if c0 < D:
                        r = r * (SCALE / LN2)
                    rb = r.astype(bf)
                    if c0 >= D:
                        ru = _tou(rb)
                        for p in range(w // 128):
                            kv_v[(c0 - D) // 128 + p, _ds(i, 128), :] = ru[:, p * 128:(p + 1) * 128]
                    if not (sub == QU - 1 and c0 == 2944):
                        qkvT_v[c0 // 2:(c0 + w) // 2, rows] = _tou(rb.T)
            if isinstance(ii, int):
                do_ln(6, qgates[2:8])
                do_ln(7, qgates[10:16])
            return c

        phase_q(0, 0)
        lax.fori_loop(1, 8 // QU, phase_q, 0)
        late_vt(7)

        def attention(s_buf0, s_buf1, p_buf0, p_buf1, m_buf, dos_buf, dl_buf, dk_acc, dv_acc, ds_buf):
            for r in (dk_acc, dv_acc, ds_buf):
                r[...] = jnp.zeros_like(r)
            s_bufs = (s_buf0, s_buf1)
            p_bufs = (p_buf0, p_buf1)
            lane_h = lax.broadcasted_iota(jnp.int32, (64, 128), 1) // 32

            def bc8(v):
                return jnp.broadcast_to(v, (8, MQ))

            def blk(b, rel):
                if isinstance(b, int):
                    b = min(max(b, 0), NBLK - 1)
                    h = b // NQB
                    qb = b % NQB
                    return dict(g=h // 4, r=h % 4, q=pl.ds(qb * MQ, MQ), s=rel % 2,
                                g64=pl.ds((h // 4) * 64, 64),
                                row=lambda base: pl.ds(base + h * 16, 16),
                                first=(qb == 0), last=(qb == NQB - 1), cache={})
                h = jnp.clip(b, 0, NBLK - 1) // NQB
                qb = rel % NQB
                return dict(g=h // 4, r=h % 4, q=pl.ds(qb * MQ, MQ), s=rel % 2,
                            g64=pl.ds(pl.multiple_of((h // 4) * 64, 64), 64),
                            row=lambda base: pl.ds(pl.multiple_of(base + h * 16, 16), 16),
                            first=(qb == 0), last=(qb == NQB - 1), cache={})

            def accum(first, acc_ref, ks, new):
                return new if first else acc_ref[:, ks] + new

            def steps(get_blk, tau0, n, st, pos_max):
                def do_dkdq(c, j, dsb):
                    ks = slice(j * KC, (j + 1) * KC)
                    if 'qT' not in c['cache']:
                        c['cache']['qT'] = _tobf(qkvT_v[c['row'](0), c['q']])
                    dk_new = accum(c['first'], dk_acc, ks, _dot(c['cache']['qT'], dsb, NT))
                    if not c['last']:
                        dk_acc[:, ks] = dk_new
                    if c['last']:
                        dqkvT_v[c['row'](512), ks] = _tou((dk_new * LN2).astype(bf))
                    kT = _tobf(qkvT_v[c['row'](512), ks])
                    dq = _dot(kT, dsb, NN)
                    st['dq'] = dq if j == 0 else st['dq'] + dq
                    if j == NCH - 1:
                        dqkvT_v[c['row'](0), c['q']] = _tou((st['dq'] * SCALE).astype(bf))

                for tau in range(tau0, tau0 + n):
                    pos_b = tau + LEAD_B
                    do_b = 0 <= pos_b < pos_max
                    if do_b:
                        b = get_blk(pos_b // NCH)
                        jb = pos_b % NCH
                        mb = m_buf[b['s']]
                        if st['cm'] is not None:
                            mb = _after(mb, st['cm'], zero_v[...])
                        p = jnp.exp2(_sub8(s_bufs[b['s']][jb * KC:(jb + 1) * KC, :], mb))
                        acc = p[KC - 8:KC] if jb == 0 else st['l'] + p[KC - 8:KC]
                        for i in range(KC // 8 - 2, -1, -1):
                            acc = acc + p[i * 8:(i + 1) * 8]
                        st['l'] = acc
                        pbn = p.astype(bf)
                        p_bufs[b['s']][jb * 64:(jb + 1) * 64, :] = _tou(pbn)
                    if tau >= 0:
                        c = get_blk(tau // NCH)
                        j = tau % NCH
                        ks = slice(j * KC, (j + 1) * KC)
                        ksu = slice(j * 64, (j + 1) * 64)
                        if 'dosT' not in c['cache']:
                            c['cache']['dosT'] = _tobf(dos_buf[c['s']])
                            c['cache']['dos4'] = jnp.concatenate([c['cache']['dosT']] * 4, axis=0)
                            c['cache']['dl'] = dl_buf[c['s']]
                        v4 = _tobf(jnp.where(lane_h == c['r'], kv_v[8 + c['g'], ksu, :], jnp.uint32(0)))
                        dpT = _dot(v4, c['cache']['dos4'], NN)
                        pb = _tobf(p_bufs[c['s']][ksu, :])
                        dv_new = accum(c['first'], dv_acc, ks, _dot(c['cache']['dosT'], pb, NT))
                        if not c['last']:
                            dv_acc[:, ks] = dv_new
                        if c['last']:
                            dqkvT_v[c['row'](1024), ks] = _tou(dv_new.astype(bf))
                        dsb = (pb.astype(f32) * _sub8(dpT, c['cache']['dl'])).astype(bf)
                        if st['pend'] is not None:
                            do_dkdq(*st['pend'])
                        st['pend'] = (c, j, dsb)
                    pos_a = tau + LEAD_A
                    if pos_a < pos_max:
                        a = get_blk(pos_a // NCH)
                        ja = pos_a % NCH
                        kau = slice(ja * 64, (ja + 1) * 64)
                        k4 = _tobf(jnp.where(lane_h == a['r'], kv_v[a['g'], kau, :], jnp.uint32(0)))
                        sT = _dot(k4, _tobf(qkvT_v[a['g64'], a['q']]), NN)
                        s_bufs[a['s']][ja * KC:(ja + 1) * KC, :] = sT
                        cm = jnp.max(_r3(sT), axis=0)
                        st['cm'] = cm
                        st['m'] = cm if ja == 0 else jnp.maximum(st['m'], cm)
                        if ja == NCH - 1:
                            m_buf[a['s']] = bc8(jnp.max(st['m'], axis=0, keepdims=True))
                    else:
                        st['cm'] = dpT[0:8]
                    if do_b:
                        vT = _tobf(qkvT_v[b['row'](1024), jb * KC:(jb + 1) * KC])
                        o = _dot(vT, pbn, NN)
                        st['ot'] = o if jb == 0 else st['ot'] + o
                        if jb == NCH - 1:
                            rl = 1.0 / jnp.sum(st['l'], axis=0, keepdims=True)
                            ot = st['ot'] * rl
                            oT_v[b['row'](0), b['q']] = _tou(ot.astype(bf))
                            dob = _tobf(dOT_v[b['row'](0), b['q']]).astype(f32) * rl
                            dos_buf[b['s']] = _tou(dob.astype(bf))
                            dl_buf[b['s']] = bc8(jnp.sum(dob * ot, axis=0, keepdims=True))
                return do_dkdq

            def blk_getter(base):
                cache = {}

                def get(rb):
                    if rb not in cache:
                        cache[rb] = blk(base + rb, rb)
                    return cache[rb]

                return get

            nstep = UB * NCH
            nit = NBLK // UB - 1
            big = 1 << 30
            st = dict(m=None, l=None, ot=None, dq=None, pend=None, cm=None)
            steps(blk_getter(0), -LEAD_A, LEAD_A, st, big)

            def body(it, carry):
                m, l, ot, dq = carry
                get = blk_getter(it * UB)
                st = dict(m=m, l=l, ot=ot, dq=dq, cm=None, pend=(get(-1), NCH - 1, _tobf(ds_buf[...])))
                steps(get, 0, nstep, st, big)
                ds_buf[...] = _tou(st['pend'][2])
                return st['m'], st['l'], st['ot'], st['dq']

            m, l, ot, dq = lax.fori_loop(
                0, nit, body, (st['m'], st['l'], st['ot'], jnp.zeros((32, MQ), f32)))
            get = blk_getter(0)
            t0 = nit * nstep
            st = dict(m=m, l=l, ot=ot, dq=dq, cm=None,
                      pend=(get(t0 // NCH - 1), NCH - 1, _tobf(ds_buf[...])))
            fin = steps(get, t0, nstep, st, NBLK * NCH)
            fin(*st['pend'])

        pl.run_scoped(
            attention,
            pltpu.VMEM((S, MQ), f32), pltpu.VMEM((S, MQ), f32),
            pltpu.VMEM((S // 2, MQ), u32), pltpu.VMEM((S // 2, MQ), u32),
            pltpu.VMEM((2, 8, MQ), f32), pltpu.VMEM((2, 16, MQ), u32), pltpu.VMEM((2, 8, MQ), f32),
            pltpu.VMEM((32, S), f32), pltpu.VMEM((32, S), f32), pltpu.VMEM((64, MQ), u32),
        )

        def phase_w(i, c):
            acq_wo(i)
            acq_wq(i)
            for k in range(rt // 256):
                rows = pl.ds(pl.multiple_of(i * rt + k * 256, 256), 256)
                dq_b = _tobf(dqkvT_v[:, rows])
                for m in range(4):
                    r = _dot(wqkv_v[m * 256:(m + 1) * 256, :], dq_b, NN)
                    dxa_v[rows, m * 256:(m + 1) * 256] = r.T
            oTb = _tobf(oT_v[_ds(i, ro // 2), :])
            onat_v[:, _ds(i, ro)] = _tou(oTb.T)
            st_wo[i % 2] = _dot(oTb, dout_v[...], NN).astype(bf)
            rel_wo(i)
            st_wqkv[i % 2] = _dot(_tobf(xnT_v[...]), _tobf(dqkvT_v[_ds(i, cq // 2), :]), NT).astype(bf)
            rel_wq(i)
            return c

        lax.fori_loop(0, WI, phase_w, 0)

    pl.run_scoped(
        scope_a,
        pltpu.VMEM((D, 3 * D), bf),
        pltpu.VMEM((16, S // 2, 128), u32),
        pltpu.VMEM((3 * D // 2, S), u32),
        pltpu.VMEM((D // 2, S), u32),
        pltpu.VMEM((D // 2, S), u32),
        pltpu.VMEM((3 * D // 2, S), u32),
    )

    def scope_b(wsp_v, wout_v, z1_v, z2_v, gp_v, uT_v, wspT_v, rs2_v, db_v, bs_v, zf_v,
                st_a, st_b, st_c, st_d, st_e):
        in_copy(wsp_hbm, wsp_v, SEM_WSP).start()
        in_copy(wout_hbm, wout_v, SEM_WOUT).start()
        in_copy(bsp_hbm, bs_v.at[pl.ds(0, 16)], SEM_B).start()
        in_copy(win_hbm, win_v, SEM_WIN).wait()

        def phase_p1(ii, c):
            for sub in range(P1U):
                i = ii * P1U + sub
                ru = _ds(i, 128)
                xnb = _tobf(xn_v[ru, :])
                zf = zf_v.at[sub]
                s1 = None
                for n in range(7):
                    cs = slice(FH + n * 256, FH + (n + 1) * 256)
                    z, dz = _gelu_and_grad(_dot(xnb, win_v[:, cs], NN))
                    gp_v[ru, cs] = _tou(dz.astype(bf))
                    zf[:, n * 256:(n + 1) * 256] = z
                    s1 = _fold128(z) if s1 is None else s1 + _fold128(z)
                gates = []
                for c0, w in [(n * 256, 256) for n in range(6)] + [(1536, 128), (1664, 128)]:
                    cs = slice(c0, c0 + w)
                    pre = _dot(xnb, win_v[:, cs], NN)
                    gates += [pre[:, t * 128:(t + 1) * 128] for t in range(w // 128)]
                    z, dz = _gelu_and_grad(pre)
                    gp_v[ru, cs] = _tou(dz.astype(bf))
                    z1_v[ru, cs] = _tou(z.astype(bf))
                zero = zero_v[:, :128]
                m = _after(_lanesum_b(s1, 1.0 / FH), _spread(gates[1:7], 32), zero)
                s2 = None
                for t in range(FH // 128):
                    zc = zf[:, t * 128:(t + 1) * 128] - m
                    s2 = zc * zc if s2 is None else s2 + zc * zc
                rstd = lax.rsqrt(_lanesum_b(s2, 1.0 / FH) + EPS)
                rs2_v[_ds(i, 256), :] = rstd
                rstd = _after(rstd, _spread(gates[8:13], 32), zero)
                mr = m * rstd
                for t in range(FH // 128):
                    ts = slice(t * 128, (t + 1) * 128)
                    z2_v[ru, ts] = _tou((zf[:, ts] * rstd - mr).astype(bf))
            return c

        lax.fori_loop(0, 8 // P1U, phase_p1, 0)

        in_copy(wsp_hbm, wsp_v, SEM_WSP).wait()
        in_copy(wout_hbm, wout_v, SEM_WOUT).wait()
        n2 = S // R2
        in_copy(bsp_hbm, bs_v.at[pl.ds(0, 16)], SEM_B).wait()
        db_v[0:16, :] = bs_v[0:16, :].astype(f32)
        acq_o, rel_o, drain_o = stream_out(n2, st_a, lambda i: out_hbm.at[_ds(i, R2)], SEM_ST)
        acq_s, rel_s, drain_s = stream_out(4, st_b, lambda i: dwsp_hbm.at[_ds(i, 512)], SEM_ST + 2)

        def phase_p2(i, c):
            acq_o(i)
            rows = _ds(i, R2)
            ru = _ds(i, R2 // 2)
            wsp_b = wsp_v[rows, :]
            wspT_v[:, rows] = _tou(wsp_b.T)
            dout_b = dout_v[rows, :]
            bcol = jnp.concatenate(
                [jnp.broadcast_to(db_v[pl.ds(i * (R2 // 128) + t, 1), :], (128, 128)).T
                 for t in range(R2 // 128)], axis=0)
            bcol2 = jnp.concatenate([bcol, bcol], axis=1)
            us = []
            dbacc = None
            for n in range(7):
                cs = slice(n * 256, (n + 1) * 256)
                g = _dot(wsp_b, _tobf(z2_v[:, cs]), NN) + bcol2
                du = _dot(dout_b, wout_v[cs, :], NT)
                z1 = _tobf(z1_v[ru, cs]).astype(f32)
                ub = (z1 * g).astype(bf)
                dg = du * z1
                part = dg[:, :128] + dg[:, 128:]
                dbacc = part if dbacc is None else dbacc + part
                dgb = dg.astype(bf)
                z1_v[ru, cs] = _tou(dgb)
                gp1 = _tobf(gp_v[ru, cs]).astype(f32)
                gp_v[ru, cs] = _tou((du * g * gp1).astype(bf))
                uT_v[n * 128:(n + 1) * 128, rows] = _tou(ub.T)
                us.append(ub)
            acc = _dot(_tobf(onat_v[ru, :]), wo_v[...], NN)
            acc = acc + _dot(jnp.concatenate(us, axis=1), wout_v[...], NN)
            st_a[i % 2] = (x_v[rows, :].astype(f32) + acc).astype(bf)
            rel_o(i)
            for t in range(R2 // 128):
                db_v[pl.ds(i * (R2 // 128) + t, 1), :] = jnp.sum(
                    dbacc[t * 128:(t + 1) * 128].T, axis=0, keepdims=True)
            return c

        def phase_p2b(i, c):
            acq_s(i)
            st_b[i % 2] = _dot(_tobf(z1_v[_ds(i, 256), :]), _tobf(z2_v[...]), NT).astype(bf)
            rel_s(i)
            return c

        lax.fori_loop(0, n2, phase_p2, 0)
        lax.fori_loop(0, 4, phase_p2b, 0)
        bs_v[0:16, :] = db_v[0:16, :].astype(bf)
        in_copy(bs_v.at[pl.ds(0, 16)], dbsp_hbm, SEM_B).start()

        n3 = S // R3
        rw = FH // n3
        acq_x, rel_x, drain_x = stream_out(n3, st_c, lambda i: dx_hbm.at[_ds(i, R3)], SEM_ST + 4)
        acq_w, rel_w, drain_w = stream_out(n3, st_d, lambda i: dwout_hbm.at[_ds(i, rw)], SEM_ST + 6)

        def phase_p3(i, c):
            acq_x(i)
            acq_w(i)
            rows = _ds(i, R3)
            ru = _ds(i, R3 // 2)
            wb = _tobf(wspT_v[ru, :])
            dyf = zf_v.at[0, :R3]
            sa = sb = None
            for n in range(7):
                cs = slice(n * 256, (n + 1) * 256)
                dy = _dot(wb, _tobf(z1_v[:, cs]), NN)
                dyf[:, cs] = dy
                pa = _fold128(dy)
                pb = _fold128(dy * _tobf(z2_v[ru, cs]).astype(f32))
                sa = pa if sa is None else sa + pa
                sb = pb if sb is None else sb + pb
            zero = zero_v[:, :128]
            dp1 = _tobf(gp_v[ru, :FH])
            dxn1 = [_dot(dp1, win_v[n * 256:(n + 1) * 256, :FH], NT) for n in range(4)]
            rstd2 = rs2_v[rows, :]
            gate = _spread([d[:, t * 128:(t + 1) * 128] for d in dxn1[:3] for t in range(2)], R3 // 8)
            ra = _lanesum_b(_after(sa, gate, zero), 1.0 / FH)
            rb = _lanesum_b(_after(sb, gate, zero), 1.0 / FH)
            dp2 = []
            for t in range(FH // 128):
                ts = slice(t * 128, (t + 1) * 128)
                gs = slice(FH + t * 128, FH + (t + 1) * 128)
                dz2 = ((dyf[:, ts] - ra) - _tobf(z2_v[ru, ts]).astype(f32) * rb) * rstd2
                d = (dz2 * _tobf(gp_v[ru, gs]).astype(f32)).astype(bf)
                gp_v[ru, gs] = _tou(d)
                dp2.append(d)
            dp2 = jnp.concatenate(dp2, axis=1)
            dxf = zf_v.at[1, :R3]
            sa = sb = None
            for n in range(4):
                cs = slice(n * 256, (n + 1) * 256)
                dxn = (dxa_v[rows, cs] + dxn1[n]) + _dot(dp2, win_v[cs, FH:], NT)
                dxf[:, cs] = dxn
                pa = _fold128(dxn)
                pb = _fold128(dxn * _tobf(xn_v[ru, cs]).astype(f32))
                sa = pa if sa is None else sa + pa
                sb = pb if sb is None else sb + pb
            uTb = _tobf(uT_v[_ds(i, rw // 2), :])
            dwo = [_dot(uTb, dout_v[:, n * 256:(n + 1) * 256], NN) for n in range(4)]
            for n in range(4):
                st_d[i % 2, :, n * 256:(n + 1) * 256] = dwo[n].astype(bf)
            gate = _spread([d[:, t * 128:(t + 1) * 128] for d in dwo[:3] for t in range(2)], R3 // 8)
            rstd = rsx_v[rows, :]
            ra = _lanesum_b(_after(sa, gate, zero), 1.0 / D)
            rb = _lanesum_b(_after(sb, gate, zero), 1.0 / D)
            for t in range(D // 128):
                ts = slice(t * 128, (t + 1) * 128)
                dx = (((dxf[:, ts] - ra) - _tobf(xn_v[ru, ts]).astype(f32) * rb) * rstd
                      + dout_v[rows, ts].astype(f32))
                st_c[i % 2, :, ts] = dx.astype(bf)
            rel_x(i)
            rel_w(i)
            return c

        lax.fori_loop(0, n3, phase_p3, 0)

        n4 = F // C4
        np4 = C4 // 128

        def cp4(i, k):
            return pltpu.make_async_copy(
                st_e.at[i % 2, k], dwin_hbm.at[:, pl.ds(pl.multiple_of(i * C4 + k * 128, 128), 128)],
                sems.at[SEM_ST + 8 + (i % 2) * np4 + k])

        def drain_i():
            for i in (n4 - 2, n4 - 1):
                for k in range(np4):
                    cp4(i, k).wait()

        def phase_p4(i, c):
            @pl.when(i >= 2)
            def _():
                for k in range(np4):
                    cp4(i - 2, k).wait()

            xnT = _tobf(xnT_v[...])
            for k in range(np4):
                cols = pl.ds(pl.multiple_of(i * C4 + k * 128, 128), 128)
                st_e[i % 2, k] = _dot(xnT, _tobf(gp_v[:, cols]), NN).astype(bf)
                cp4(i, k).start()
            return c

        lax.fori_loop(0, n4, phase_p4, 0)
        in_copy(bs_v.at[pl.ds(0, 16)], dbsp_hbm, SEM_B).wait()
        drain_wo()
        drain_wq()
        drain_o()
        drain_s()
        drain_x()
        drain_w()
        drain_i()

    pl.run_scoped(
        scope_b,
        pltpu.VMEM((S, S), bf),
        pltpu.VMEM((FH, D), bf),
        pltpu.VMEM((S // 2, FH), u32),
        pltpu.VMEM((S // 2, FH), u32),
        pltpu.VMEM((S // 2, F), u32),
        pltpu.VMEM((FH // 2, S), u32),
        pltpu.VMEM((S // 2, S), u32),
        pltpu.VMEM((S, 128), f32),
        pltpu.VMEM((32, 128), f32),
        pltpu.VMEM((64, 128), bf),
        pltpu.VMEM((2, 256, FH), f32),
        pltpu.VMEM((2, R2, D), bf),
        pltpu.VMEM((2, 512, S), bf),
        pltpu.VMEM((2, R3, D), bf),
        pltpu.VMEM((2, FH * R3 // S, D), bf),
        pltpu.VMEM((2, C4 // 128, D, 128), bf),
    )


@jax.jit
def pallas_parallel_sum__mha_block__mixer_gmlp__prompt_kernel(
    A_x: jax.Array,
    A_wqkv: jax.Array,
    A_wo: jax.Array,
    B_x: jax.Array,
    B_w_in: jax.Array,
    B_w_sp: jax.Array,
    B_b_sp: jax.Array,
    B_w_out: jax.Array,
    grad_out: jax.Array,
):
    del B_x
    any_spec = pl.BlockSpec(memory_space=pl.ANY)
    out_shape = (
        jax.ShapeDtypeStruct((S, D), bf),
        jax.ShapeDtypeStruct((S, D), bf),
        jax.ShapeDtypeStruct((D, 3 * D), bf),
        jax.ShapeDtypeStruct((D, D), bf),
        jax.ShapeDtypeStruct((D, F), bf),
        jax.ShapeDtypeStruct((S, S), bf),
        jax.ShapeDtypeStruct((S // 128, 128), bf),
        jax.ShapeDtypeStruct((FH, D), bf),
    )
    outs = pl.pallas_call(
        _kernel,
        out_shape=out_shape,
        in_specs=[any_spec] * 8,
        out_specs=(any_spec,) * 8,
        scratch_shapes=[
            pltpu.VMEM((S, D), bf),
            pltpu.VMEM((S, D), bf),
            pltpu.VMEM((D, D), bf),
            pltpu.VMEM((D, F), bf),
            pltpu.VMEM((S // 2, D), u32),
            pltpu.VMEM((D // 2, S), u32),
            pltpu.VMEM((S // 2, D), u32),
            pltpu.VMEM((S, D), f32),
            pltpu.VMEM((S, 128), f32),
            pltpu.VMEM((8, MQ), u32),
            pltpu.VMEM((2, D // WI, D), bf),
            pltpu.VMEM((2, D, 3 * D // WI), bf),
            pltpu.SemaphoreType.DMA((NSEM,)),
        ],
        compiler_params=pltpu.CompilerParams(vmem_limit_bytes=127 * 1024 * 1024),
        name="mha_gmlp_fwd_bwd",
    )(
        A_x.reshape(S, D), A_wqkv, A_wo, B_w_in, B_w_sp, B_b_sp.reshape(S // 128, 128), B_w_out,
        grad_out.reshape(S, D),
    )
    out, dx, dwqkv, dwo, dwin, dwsp, dbsp, dwout = outs
    return (out.reshape(1, S, D), dx.reshape(1, S, D), dwqkv, dwo, dwin, dwsp,
            dbsp.reshape(S), dwout)
```
